```python
import jax
import jax.numpy as jnp

def _softmax(x, axis=-1):
    return jax.nn.softmax(x, axis=axis)
def _gelu(x):
    return jax.nn.gelu(x, approximate=True)
def _silu(x):
    return jax.nn.silu(x)
def _sigmoid(x):
    return jax.nn.sigmoid(x)
def _layernorm(x, axis=-1, eps=1e-5):
    m = jnp.mean(x, axis=axis, keepdims=True)
    v = jnp.var(x, axis=axis, keepdims=True)
    return (x - m) / jnp.sqrt(v + eps)
def _scatter_add(tgt, idx, src, axis=0):
    return tgt.at[idx].add(src)
def _segment_sum(src, seg, n):
    return jax.ops.segment_sum(src, seg, n)
class _Rng:
    def __init__(self, key):
        self._k = key
    def _next(self):
        self._k, sub = jax.random.split(self._k)
        return sub
    def normal(self, shape):
        return jax.random.normal(self._next(), shape, dtype=jnp.bfloat16)
    def randint(self, lo, hi, shape):
        return jax.random.randint(self._next(), shape, lo, hi, dtype=jnp.int32)
    def uniform(self, shape, lo=0.0, hi=1.0):
        return jax.random.uniform(self._next(), shape, jnp.bfloat16, lo, hi)
    def permutation(self, n):
        return jax.random.permutation(self._next(), n)


kernel_name = 'standalone__seq2seq_rnn_t_joint__speech'

def setup_inputs():
    _rng = _Rng(jax.random.key(int.from_bytes(__import__("os").urandom(4), "little")))
    _w = (lambda a: (lambda t: t.astype(jnp.bfloat16) if jnp.issubdtype(t.dtype, jnp.floating) else t)(jnp.asarray(a)))
    B, T, D, K = 2, 16000, 256, 31
    U = 8
    sc = (1.0 / (K * D)) ** 0.5
    sd = (1.0 / D) ** 0.5
    return {
        "x": _w((lambda *s: _rng.normal(s) * 0.05)(B, T, D) * 0.5),
        "w1": _w((lambda *s: _rng.normal(s) * 0.05)(K, D, D) * sc),
        "w2": _w((lambda *s: _rng.normal(s) * 0.05)(K, D, D) * sc),
        "g": _w((lambda *s: _rng.normal(s) * 0.05)(B, U, D) * 0.5),
        "w_f": _w((lambda *s: _rng.normal(s) * 0.05)(D, D) * sd),
        "w_g": _w((lambda *s: _rng.normal(s) * 0.05)(D, D) * sd),
        "w_o": _w((lambda *s: _rng.normal(s) * 0.05)(D, D) * sd),
    }

def reference(x, w1, w2, g, w_f, w_g, w_o):
    B, T, D = x.shape
    K = w1.shape[0]
    pad = K // 2
    xp = jnp.pad(x, ((0,0),(pad,pad),(0,0)))
    h = jnp.zeros_like(x)
    for i in range(K):
        h = h + jnp.einsum("btc,cd->btd", xp[:, i:i+T, :], w1[i])
    h = _gelu(h)[:, ::2, :]
    T1 = h.shape[1]
    hp = jnp.pad(h, ((0,0),(pad,pad),(0,0)))
    f = jnp.zeros_like(h)
    for i in range(K):
        f = f + jnp.einsum("btc,cd->btd", hp[:, i:i+T1, :], w2[i])
    f = _gelu(f)[:, ::2, :]
    fe = jnp.einsum("btd,de->bte", f, w_f)
    ge = jnp.einsum("bud,de->bue", g, w_g)
    j = jnp.tanh(fe[:, :, None, :] + ge[:, None, :, :])
    return jnp.einsum("btud,dv->btuv", j, w_o)
```

```python
import itertools

import numpy as np
import jax
import jax.numpy as jnp
from jax import lax
from jax.experimental import pallas as pl
from jax.experimental.pallas import tpu as pltpu

f32, bf16, u32, i32 = jnp.float32, jnp.bfloat16, jnp.uint32, jnp.int32

B, T, D, K, U = 2, 16000, 256, 31, 8
T1, T2 = T // 2, T // 4
NSEG = 16
G = 4
MB = G * NSEG
P1 = 532
P2 = 274
P3 = 132
NB1, NB2 = 8, 4
XPART = (0, 80, 208, 336, 528)
WPIECE = 4
NDOT = 162
LEAD = 6
_C0 = np.float32(np.sqrt(2.0 / np.pi))
_C1 = np.float32(0.044715)
_TG = ((0,), (0, 1), (1,))


def _unpack(w, i):
    return pltpu.unpack_elementwise(w, index=i, packed_dtype=bf16, unpacked_dtype=f32)


def _pack(lo, hi):
    return pltpu.pack_elementwise([lo, hi], packed_dtype=bf16)


def _gelu(x):
    return 0.5 * x * (1.0 + jnp.tanh(_C0 * (x + _C1 * x * x * x)))


def _kar(x0, x1, x2):
    return (x0 - x1, x1, x2 - x1)


def _micro(v):
    w = [_kar(v[i], v[i + 2], v[i + 4]) for i in range(3)]
    out = []
    for ka in range(3):
        out.extend(_kar(w[0][ka], w[1][ka], w[2][ka]))
    return out


def _wtree(get, n):
    if n == 1:
        yield get(0)
        return
    h = n // 2
    lo = [get(j) for j in range(h)]
    yield from _wtree(lambda j: lo[j], h)
    hi = [get(h + j) for j in range(h)]
    mid = [(lo[j][0] + hi[j][0], lo[j][1] + hi[j][1]) for j in range(h)]
    yield from _wtree(lambda j: mid[j], h)
    yield from _wtree(lambda j: hi[j], h)


def _transform_weights(w_raw, wt, piece):
    per = D // 16 // WPIECE
    for r in range(piece * per, (piece + 1) * per):
        for ph in range(2):
            for nt in range(2):
                def get(j, ph=ph, r=r, nt=nt):
                    tap = 2 * j if ph == 1 else 2 * j - 1
                    if tap < 0:
                        z = jnp.zeros((8, 128), f32)
                        return (z, z)
                    wv = pltpu.bitcast(w_raw[tap, pl.ds(16 * r, 16), pl.ds(128 * nt, 128)], u32)
                    return (_unpack(wv, 0), _unpack(wv, 1))
                for k, (lo, hi) in enumerate(_wtree(get, 16)):
                    wt[k, pl.ds(ph * 128 + 8 * r, 8), pl.ds(128 * nt, 128)] = _pack(lo, hi)


def _input_units(load, t_out):
    u = {}

    def p1(gq, lt, h, p):
        def run():
            ws = [load(gq, lt, h, p + 4 * j) for j in range(7)]
            for ph in range(2):
                o = _micro([_unpack(w, ph) for w in ws])
                for k in range(9):
                    u[gq, lt, ph, h, k, p] = o[k]
        return run

    def p2(gq, lt, ph, ka):
        def run():
            oa = _micro([u.pop((gq, lt, ph, 0, ka, p)) for p in range(7)])
            ob = _micro([u.pop((gq, lt, ph, 1, ka, p)) for p in range(7)])
            for kb in range(9):
                t_out[ka * 9 + kb, pl.ds(gq * 8, 8), pl.ds(ph * 256 + lt * 128, 128)] = _pack(oa[kb], ob[kb])
        return run

    cols = [(gq, lt) for gq in range(G) for lt in range(2)]
    seq = []
    for ci in range(len(cols) + 1):
        a = [p1(*cols[ci], h, p) for h in range(2) for p in range(7)] if ci < len(cols) else []
        b = [p2(*cols[ci - 1], ph, ka) for ph in range(2) for ka in range(9)] if ci > 0 else []
        ia = ib = 0
        while ia < len(a) or ib < len(b):
            if ib >= len(b) or (ia < len(a) and ia * len(b) <= ib * len(a)):
                seq.append(a[ia]); ia += 1
            else:
                seq.append(b[ib]); ib += 1
    return seq


def _conv_block(t_in, wt, acc, store, units):
    st = [0, 0]

    def tick():
        st[1] += 1
        want = min(len(units), -(-(st[1] * len(units)) // (NDOT - LEAD)))
        while st[0] < want:
            units[st[0]]()
            st[0] += 1

    groups = list(itertools.product(range(3), repeat=3))
    last = {}
    for gi, (k3, k2, k1) in enumerate(groups):
        for t in itertools.product(_TG[k3], _TG[k2], _TG[k1]):
            last[t] = gi
    seen = set()
    for gi, (k3, k2, k1) in enumerate(groups):
        k = (k3 * 9 + k2 * 3 + k1) * 3
        for nt in range(2):
            cols = slice(nt * 128, (nt + 1) * 128)
            m = []
            for k0 in range(3):
                lhs = pltpu.bitcast(t_in[k + k0], bf16)
                rhs = pltpu.bitcast(wt[k + k0, :, cols], bf16)
                m.append(jnp.dot(lhs, rhs, preferred_element_type=f32))
                tick()
            r = (m[0] + m[1], m[1] + m[2])
            for t in itertools.product(_TG[k3], _TG[k2], _TG[k1]):
                a = t[0] * 8 + t[1] * 4 + t[2] * 2
                vals = []
                for a0 in range(2):
                    v = r[a0] if (a + a0, nt) not in seen else acc[a + a0, :, cols] + r[a0]
                    seen.add((a + a0, nt))
                    if last[t] == gi:
                        vals.append(_gelu(v))
                    else:
                        acc[a + a0, :, cols] = v
                if last[t] == gi:
                    for v in range(MB // 8):
                        store(nt, v, a // 2, _pack(vals[0][8 * v:8 * v + 8], vals[1][8 * v:8 * v + 8]))
    while st[0] < len(units):
        units[st[0]]()
        st[0] += 1


def _kernel(zero_ref, x_hbm, w1_hbm, w2_hbm, g_ref, wf_ref, wg_ref, wo_ref, out_hbm,
            rx, rh, rf, t0, t1, wraw, wt1, wt2, acc0, wfp, wop, ge, ob, mode,
            sem_w, sem_x, sem_o):
    zero = zero_ref[0]
    acc = acc0.at[pl.ds(zero, 16)]
    rxw = rx.bitcast(u32)

    def x_copies(b, part):
        cps = []
        lo, hi = XPART[part], XPART[part + 1]
        for s in range(NSEG):
            q0 = max(512 * s - 8 + lo, 0)
            q1 = min(512 * s - 8 + hi, T1)
            if q1 <= q0:
                continue
            loc = q0 - (512 * s - 8)
            for lt in range(2):
                cps.append(pltpu.make_async_copy(
                    x_hbm.at[b, pl.ds(2 * q0, 2 * (q1 - q0)), pl.ds(128 * lt, 128)],
                    rx.at[lt, s % 2, pl.ds(2 * (P1 * (s // 2) + loc), 2 * (q1 - q0)), :],
                    sem_x.at[part]))
        return cps

    def w_copy(w_hbm, i, piece):
        rows = pl.ds(piece * (D // WPIECE), D // WPIECE)
        return pltpu.make_async_copy(w_hbm.at[:, rows, :], wraw.at[i, :, rows, :], sem_w.at[i * WPIECE + piece])

    def out_copy(slot, s, rows, b, t0_):
        return pltpu.make_async_copy(
            ob.at[slot, s, pl.ds(0, rows)], out_hbm.at[b, pl.ds(t0_, rows)], sem_o.at[slot])

    def out_wait(slot):
        m = mode[slot]

        @pl.when(m >= 0)
        def _():
            for s in range(NSEG - 1):
                out_copy(slot, s, 64, 0, 0).wait()

        @pl.when(m == 64)
        def _():
            out_copy(slot, NSEG - 1, 64, 0, 0).wait()

        @pl.when(m == 32)
        def _():
            out_copy(slot, NSEG - 1, 32, 0, 0).wait()

    w_copy(w1_hbm, 0, 0).start()
    for c in x_copies(0, 0):
        c.start()
    for piece in range(1, WPIECE):
        w_copy(w1_hbm, 0, piece).start()

    mode[0] = -1
    mode[1] = -1
    zb = jnp.zeros((16, 128), bf16)
    zw = jnp.zeros((8, 128), u32)
    for lt in range(2):
        rx[lt, 0, pl.ds(0, 16), :] = zb
        rx[lt, 1, pl.ds(2 * P1 * 7 + 656, 400), :] = jnp.zeros((400, 128), bf16)
        rh[lt, pl.ds(0, 8), :] = zw
    wfp[...] = pltpu.bitcast(wf_ref[...], u32)
    wop[...] = pltpu.bitcast(wo_ref[...], u32)
    for b in range(B):
        ge[pl.ds(8 * b, 8), :] = jnp.dot(g_ref[b], wg_ref[...], preferred_element_type=f32)

    for piece in range(WPIECE):
        w_copy(w1_hbm, 0, piece).wait()
        if piece == WPIECE - 1:
            for part in range(1, 4):
                for c in x_copies(0, part):
                    c.start()
                if part == 1:
                    for p2 in range(WPIECE):
                        w_copy(w2_hbm, 1, p2).start()
        _transform_weights(wraw.at[0], wt1, piece)

    def load_x(base):
        def load(gq, lt, h, c):
            view = rxw.at[lt, h, pl.ds(pl.multiple_of(base, 16), 7 * P1 + 80), :]
            return view[pl.ds(16 * gq + c, 8, stride=P1), :]
        return load

    def load_h(base):
        def load(gq, lt, h, c):
            view = rh.at[lt, pl.ds(pl.multiple_of(base, 64), 15 * P2 + 80), :]
            return view[pl.ds(h * P2 + 16 * gq + c, 8, stride=2 * P2), :]
        return load

    def store_h(base):
        def store(nt, v, half_a, val):
            view = rh.at[nt, pl.ds(pl.multiple_of(base, 32), 15 * P2 + 48), :]
            view[pl.ds(8 * (v % 2) * P2 + 8 + 8 * (v // 2) + half_a, 8, stride=P2), :] = val
        return store

    def store_f(base):
        def store(nt, v, half_a, val):
            view = rf.at[nt, pl.ds(pl.multiple_of(base, 32), 15 * P3 + 32), :]
            view[pl.ds(8 * (v % 2) * P3 + 8 * (v // 2) + half_a, 8, stride=P3), :] = val
        return store

    def joint_block(fbase, slot, b, blk):
        out_wait(slot)
        wf = pltpu.bitcast(wfp[...], bf16)
        wo = pltpu.bitcast(wop[...], bf16)
        geb = ge[pl.ds(pl.multiple_of(8 * b, 8), 8), :]

        def fe_of(s):
            lhs = jnp.concatenate(
                [pltpu.bitcast(rf.at[lt, pl.ds(pl.multiple_of(fbase, 32), 15 * P3 + 32), :][pl.ds(s * P3, 32), :], bf16)
                 for lt in range(2)], axis=1)
            return jnp.dot(lhs, wf, preferred_element_type=f32)

        def start_out(s):
            if s < NSEG - 1:
                out_copy(slot, s, 64, b, 256 * s + 64 * blk).start()
                return

            @pl.when(blk < 2)
            def _():
                out_copy(slot, s, 64, b, 256 * s + 64 * blk).start()

            @pl.when(blk == 2)
            def _():
                out_copy(slot, s, 32, b, 256 * s + 128).start()

        fe_next = fe_of(0)
        for s in range(NSEG):
            fe = fe_next
            if s + 1 < NSEG:
                fe_next = fe_of(s + 1)
            for c0 in range(0, 64, 16):
                if c0 == 16 and s > 0:
                    start_out(s - 1)
                rows = [jnp.tanh(jnp.broadcast_to(fe[t:t + 1, :], (8, D)) + geb) for t in range(c0, c0 + 16)]
                j = jnp.concatenate(rows, axis=0).astype(bf16)
                o = jnp.dot(j, wo, preferred_element_type=f32)
                ob[slot, s, pl.ds(c0, 16)] = o.astype(bf16).reshape(16, U, D)
        start_out(NSEG - 1)
        mode[slot] = jnp.where(blk < 2, 64, jnp.where(blk == 2, 32, 0))

    def run_units(units):
        for u in units:
            u()

    def batch(b, carry):
        for c in x_copies(b, 0):
            c.wait()
        run_units(_input_units(load_x(zero), t0))

        def conv1_step(n, c):
            xn, hc = c
            for part, step in ((1, 0), (2, 2), (3, 4)):
                @pl.when(n == step)
                def _(part=part):
                    for cp in x_copies(b, part):
                        cp.wait()

            @pl.when(n % 2 == 0)
            def _():
                _conv_block(t0, wt1, acc, store_h(hc), _input_units(load_x(xn), t1))

            @pl.when(n % 2 == 1)
            def _():
                _conv_block(t1, wt1, acc, store_h(hc), _input_units(load_x(xn), t0))
            return (jnp.minimum(xn + 64, 64 * (NB1 - 1)), hc + 32)
        lax.fori_loop(0, NB1, conv1_step, (zero + 64, zero))

        @pl.when(b == 0)
        def _():
            for part in range(4):
                for c in x_copies(1, part):
                    c.start()
            for piece in range(WPIECE):
                w_copy(w2_hbm, 1, piece).wait()
                _transform_weights(wraw.at[1], wt2, piece)

        for lt in range(2):
            for s in range(NSEG - 1):
                rh[lt, pl.ds((s + 1) * P2, 8), :] = rh[lt, pl.ds(s * P2 + 256, 8), :]
                rh[lt, pl.ds(s * P2 + 264, 8), :] = rh[lt, pl.ds((s + 1) * P2 + 8, 8), :]
            rh[lt, pl.ds(15 * P2 + 168, 104), :] = jnp.zeros((104, 128), u32)

        run_units(_input_units(load_h(zero), t0))

        def conv2_step(n, c):
            hn, fc = c

            @pl.when(n % 2 == 0)
            def _():
                _conv_block(t0, wt2, acc, store_f(fc), _input_units(load_h(hn), t1))

            @pl.when(n % 2 == 1)
            def _():
                _conv_block(t1, wt2, acc, store_f(fc), _input_units(load_h(hn), t0))
            joint_block(fc, n % 2, b, n)
            return (jnp.minimum(hn + 64, 64 * (NB2 - 1)), fc + 32)
        lax.fori_loop(0, NB2, conv2_step, (zero + 64, zero))
        return carry

    lax.fori_loop(0, B, batch, 0)
    out_wait(0)
    out_wait(1)


def _scratch():
    return [
        pltpu.VMEM((2, 2, 2 * 8 * P1, 128), bf16),
        pltpu.VMEM((2, NSEG * P2, 128), u32),
        pltpu.VMEM((2, NSEG * P3, 128), u32),
        pltpu.VMEM((81, MB // 2, 512), u32),
        pltpu.VMEM((81, MB // 2, 512), u32),
        pltpu.VMEM((2, K, D, D), bf16),
        pltpu.VMEM((81, 256, 256), u32),
        pltpu.VMEM((81, 256, 256), u32),
        pltpu.VMEM((32, MB, D), f32),
        pltpu.VMEM((128, D), u32),
        pltpu.VMEM((128, D), u32),
        pltpu.VMEM((16, D), f32),
        pltpu.VMEM((2, NSEG, 64, U, D), bf16),
        pltpu.SMEM((2,), i32),
        pltpu.SemaphoreType.DMA((2 * WPIECE,)),
        pltpu.SemaphoreType.DMA((4,)),
        pltpu.SemaphoreType.DMA((2,)),
    ]


@jax.jit
def pallas_standalone__seq2seq_rnn_t_joint__speech_kernel(x, w1, w2, g, w_f, w_g, w_o):
    any_spec = pl.BlockSpec(memory_space=pl.ANY)
    vm = pl.BlockSpec(memory_space=pltpu.VMEM)
    return pl.pallas_call(
        _kernel,
        out_shape=jax.ShapeDtypeStruct((B, T2, U, D), bf16),
        in_specs=[pl.BlockSpec(memory_space=pltpu.SMEM), any_spec, any_spec, any_spec, vm, vm, vm, vm],
        out_specs=any_spec,
        scratch_shapes=_scratch(),
        compiler_params=pltpu.CompilerParams(vmem_limit_bytes=120 * 2 ** 20),
    )(np.zeros((1,), np.int32), x, w1, w2, g, w_f, w_g, w_o)
```

```python
import itertools

import numpy as np
import jax
import jax.numpy as jnp
from jax import lax
from jax.experimental import pallas as pl
from jax.experimental.pallas import tpu as pltpu

f32, bf16, u32, i32 = jnp.float32, jnp.bfloat16, jnp.uint32, jnp.int32

B, T, D, K, U = 2, 16000, 256, 31, 8
T1, T2 = T // 2, T // 4
NSEG = 16
G = 4
MB = G * NSEG
P1 = 532
P2 = 274
P3 = 132
NB1, NB2 = 8, 4
XPART = (0, 80, 208, 336, 528)
WPIECE = 4
NDOT = 162
LEAD = 6
_C0 = np.float32(np.sqrt(2.0 / np.pi))
_C1 = np.float32(0.044715)
_TG = ((0,), (0, 1), (1,))


def _unpack(w, i):
    return pltpu.unpack_elementwise(w, index=i, packed_dtype=bf16, unpacked_dtype=f32)


def _pack(lo, hi):
    return pltpu.pack_elementwise([lo, hi], packed_dtype=bf16)


def _gelu(x):
    return 0.5 * x * (1.0 + jnp.tanh(_C0 * (x + _C1 * x * x * x)))


def _kar(x0, x1, x2):
    return (x0 - x1, x1, x2 - x1)


def _micro(v):
    w = [_kar(v[i], v[i + 2], v[i + 4]) for i in range(3)]
    out = []
    for ka in range(3):
        out.extend(_kar(w[0][ka], w[1][ka], w[2][ka]))
    return out


def _wtree(get, n):
    if n == 1:
        yield get(0)
        return
    h = n // 2
    lo = [get(j) for j in range(h)]
    yield from _wtree(lambda j: lo[j], h)
    hi = [get(h + j) for j in range(h)]
    mid = [(lo[j][0] + hi[j][0], lo[j][1] + hi[j][1]) for j in range(h)]
    yield from _wtree(lambda j: mid[j], h)
    yield from _wtree(lambda j: hi[j], h)


def _transform_weights(w_raw, wt, piece):
    per = D // 16 // WPIECE
    for r in range(piece * per, (piece + 1) * per):
        for ph in range(2):
            for nt in range(2):
                def get(j, ph=ph, r=r, nt=nt):
                    tap = 2 * j if ph == 1 else 2 * j - 1
                    if tap < 0:
                        z = jnp.zeros((8, 128), f32)
                        return (z, z)
                    wv = pltpu.bitcast(w_raw[tap, pl.ds(16 * r, 16), pl.ds(128 * nt, 128)], u32)
                    return (_unpack(wv, 0), _unpack(wv, 1))
                for k, (lo, hi) in enumerate(_wtree(get, 16)):
                    wt[k, pl.ds(ph * 128 + 8 * r, 8), pl.ds(128 * nt, 128)] = _pack(lo, hi)


def _input_units(load, t_out):
    u = {}

    def p1(gq, lt, h, p):
        def run():
            ws = [load(gq, lt, h, p + 4 * j) for j in range(7)]
            for ph in range(2):
                o = _micro([_unpack(w, ph) for w in ws])
                for k in range(9):
                    u[gq, lt, ph, h, k, p] = o[k]
        return run

    def p2(gq, lt, ph, ka):
        def run():
            oa = _micro([u.pop((gq, lt, ph, 0, ka, p)) for p in range(7)])
            ob = _micro([u.pop((gq, lt, ph, 1, ka, p)) for p in range(7)])
            for kb in range(9):
                t_out[ka * 9 + kb, pl.ds(gq * 8, 8), pl.ds(ph * 256 + lt * 128, 128)] = _pack(oa[kb], ob[kb])
        return run

    cols = [(gq, lt) for gq in range(G) for lt in range(2)]
    seq = []
    for ci in range(len(cols) + 1):
        a = [p1(*cols[ci], h, p) for h in range(2) for p in range(7)] if ci < len(cols) else []
        b = [p2(*cols[ci - 1], ph, ka) for ph in range(2) for ka in range(9)] if ci > 0 else []
        ia = ib = 0
        while ia < len(a) or ib < len(b):
            if ib >= len(b) or (ia < len(a) and ia * len(b) <= ib * len(a)):
                seq.append(a[ia]); ia += 1
            else:
                seq.append(b[ib]); ib += 1
    return seq


def _conv_block(t_in, wt, acc, store, units):
    st = [0, 0]

    def tick():
        st[1] += 1
        want = min(len(units), -(-(st[1] * len(units)) // (NDOT - LEAD)))
        while st[0] < want:
            units[st[0]]()
            st[0] += 1

    groups = list(itertools.product(range(3), repeat=3))
    last = {}
    for gi, (k3, k2, k1) in enumerate(groups):
        for t in itertools.product(_TG[k3], _TG[k2], _TG[k1]):
            last[t] = gi
    seen = set()
    for gi, (k3, k2, k1) in enumerate(groups):
        k = (k3 * 9 + k2 * 3 + k1) * 3
        for nt in range(2):
            cols = slice(nt * 128, (nt + 1) * 128)
            m = []
            for k0 in range(3):
                lhs = pltpu.bitcast(t_in[k + k0], bf16)
                rhs = pltpu.bitcast(wt[k + k0, :, cols], bf16)
                m.append(jnp.dot(lhs, rhs, preferred_element_type=f32))
                tick()
            r = (m[0] + m[1], m[1] + m[2])
            for t in itertools.product(_TG[k3], _TG[k2], _TG[k1]):
                a = t[0] * 8 + t[1] * 4 + t[2] * 2
                vals = []
                for a0 in range(2):
                    v = r[a0] if (a + a0, nt) not in seen else acc[a + a0, :, cols] + r[a0]
                    seen.add((a + a0, nt))
                    if last[t] == gi:
                        vals.append(_gelu(v))
                    else:
                        acc[a + a0, :, cols] = v
                if last[t] == gi:
                    for v in range(MB // 8):
                        store(nt, v, a // 2, _pack(vals[0][8 * v:8 * v + 8], vals[1][8 * v:8 * v + 8]))
    while st[0] < len(units):
        units[st[0]]()
        st[0] += 1


def _kernel(zero_ref, x_hbm, w1_hbm, w2_hbm, g_ref, wf_ref, wg_ref, wo_ref, out_hbm,
            rx, rh, rf, t0, t1, wraw, wt1, wt2, acc0, wfp, wop, ge, ob, mode,
            sem_w, sem_x, sem_o):
    zero = zero_ref[0]
    acc = acc0.at[pl.ds(zero, 16)]
    rxw = rx.bitcast(u32)

    def x_copies(b, part):
        cps = []
        lo, hi = XPART[part], XPART[part + 1]
        for s in range(NSEG):
            q0 = max(512 * s - 8 + lo, 0)
            q1 = min(512 * s - 8 + hi, T1)
            if q1 <= q0:
                continue
            loc = q0 - (512 * s - 8)
            for lt in range(2):
                cps.append(pltpu.make_async_copy(
                    x_hbm.at[b, pl.ds(2 * q0, 2 * (q1 - q0)), pl.ds(128 * lt, 128)],
                    rx.at[lt, s % 2, pl.ds(2 * (P1 * (s // 2) + loc), 2 * (q1 - q0)), :],
                    sem_x.at[part]))
        return cps

    def w_copy(w_hbm, i, piece):
        rows = pl.ds(piece * (D // WPIECE), D // WPIECE)
        return pltpu.make_async_copy(w_hbm.at[:, rows, :], wraw.at[i, :, rows, :], sem_w.at[i * WPIECE + piece])

    def out_copy(slot, s, rows, b, t0_):
        return pltpu.make_async_copy(
            ob.at[slot, s, pl.ds(0, rows)], out_hbm.at[b, pl.ds(t0_, rows)], sem_o.at[slot])

    def out_wait(slot):
        m = mode[slot]

        @pl.when(m >= 0)
        def _():
            for s in range(NSEG - 1):
                out_copy(slot, s, 64, 0, 0).wait()

        @pl.when(m == 64)
        def _():
            out_copy(slot, NSEG - 1, 64, 0, 0).wait()

        @pl.when(m == 32)
        def _():
            out_copy(slot, NSEG - 1, 32, 0, 0).wait()

    w_copy(w1_hbm, 0, 0).start()
    for c in x_copies(0, 0):
        c.start()
    for piece in range(1, WPIECE):
        w_copy(w1_hbm, 0, piece).start()

    mode[0] = -1
    mode[1] = -1
    zb = jnp.zeros((16, 128), bf16)
    zw = jnp.zeros((8, 128), u32)
    for lt in range(2):
        rx[lt, 0, pl.ds(0, 16), :] = zb
        rx[lt, 1, pl.ds(2 * P1 * 7 + 656, 400), :] = jnp.zeros((400, 128), bf16)
        rh[lt, pl.ds(0, 8), :] = zw
    wfp[...] = pltpu.bitcast(wf_ref[...], u32)
    wop[...] = pltpu.bitcast(wo_ref[...], u32)
    for b in range(B):
        ge[pl.ds(8 * b, 8), :] = jnp.dot(g_ref[b], wg_ref[...], preferred_element_type=f32)

    for piece in range(WPIECE):
        w_copy(w1_hbm, 0, piece).wait()
        if piece == WPIECE - 1:
            for part in range(1, 4):
                for c in x_copies(0, part):
                    c.start()
                if part == 1:
                    for p2 in range(WPIECE):
                        w_copy(w2_hbm, 1, p2).start()
        _transform_weights(wraw.at[0], wt1, piece)

    def load_x(base):
        def load(gq, lt, h, c):
            view = rxw.at[lt, h, pl.ds(pl.multiple_of(base, 16), 7 * P1 + 80), :]
            return view[pl.ds(16 * gq + c, 8, stride=P1), :]
        return load

    def load_h(base):
        def load(gq, lt, h, c):
            view = rh.at[lt, pl.ds(pl.multiple_of(base, 64), 15 * P2 + 80), :]
            return view[pl.ds(h * P2 + 16 * gq + c, 8, stride=2 * P2), :]
        return load

    def store_h(base):
        def store(nt, v, half_a, val):
            view = rh.at[nt, pl.ds(pl.multiple_of(base, 32), 15 * P2 + 48), :]
            view[pl.ds(8 * (v % 2) * P2 + 8 + 8 * (v // 2) + half_a, 8, stride=P2), :] = val
        return store

    def store_f(base):
        def store(nt, v, half_a, val):
            view = rf.at[nt, pl.ds(pl.multiple_of(base, 32), 15 * P3 + 32), :]
            view[pl.ds(8 * (v % 2) * P3 + 8 * (v // 2) + half_a, 8, stride=P3), :] = val
        return store

    def joint_block(fbase, slot, b, blk):
        out_wait(slot)
        wf = pltpu.bitcast(wfp[...], bf16)
        wo = pltpu.bitcast(wop[...], bf16)
        geb = ge[pl.ds(pl.multiple_of(8 * b, 8), 8), :]

        def fe_of(s):
            lhs = jnp.concatenate(
                [pltpu.bitcast(rf.at[lt, pl.ds(pl.multiple_of(fbase, 32), 15 * P3 + 32), :][pl.ds(s * P3, 32), :], bf16)
                 for lt in range(2)], axis=1)
            return jnp.dot(lhs, wf, preferred_element_type=f32)

        def start_out(s):
            if s < NSEG - 1:
                out_copy(slot, s, 64, b, 256 * s + 64 * blk).start()
                return

            @pl.when(blk < 2)
            def _():
                out_copy(slot, s, 64, b, 256 * s + 64 * blk).start()

            @pl.when(blk == 2)
            def _():
                out_copy(slot, s, 32, b, 256 * s + 128).start()

        fe_next = fe_of(0)
        for s in range(NSEG):
            fe = fe_next
            if s + 1 < NSEG:
                fe_next = fe_of(s + 1)
            for c0 in range(0, 64, 16):
                if c0 == 16 and s > 0:
                    start_out(s - 1)
                rows = [jnp.tanh(jnp.broadcast_to(fe[t:t + 1, :], (8, D)) + geb) for t in range(c0, c0 + 16)]
                j = jnp.concatenate(rows, axis=0).astype(bf16)
                o = jnp.dot(j, wo, preferred_element_type=f32)
                ob[slot, s, pl.ds(c0, 16)] = o.astype(bf16).reshape(16, U, D)
        start_out(NSEG - 1)
        mode[slot] = jnp.where(blk < 2, 64, jnp.where(blk == 2, 32, 0))

    def run_units(units):
        for u in units:
            u()

    def batch(b, carry):
        for c in x_copies(b, 0):
            c.wait()
        run_units(_input_units(load_x(zero), t0))

        def conv1_step(n, c):
            xn, hc = c
            for part, step in ((1, 0), (2, 2), (3, 4)):
                @pl.when(n == step)
                def _(part=part):
                    for cp in x_copies(b, part):
                        cp.wait()

            @pl.when(n % 2 == 0)
            def _():
                _conv_block(t0, wt1, acc, store_h(hc), _input_units(load_x(xn), t1))

            @pl.when(n % 2 == 1)
            def _():
                _conv_block(t1, wt1, acc, store_h(hc), _input_units(load_x(xn), t0))
            @pl.when(n == NB1 - 1)
            def _():
                for lt in range(2):
                    for s in range(NSEG - 1):
                        rh[lt, pl.ds((s + 1) * P2, 8), :] = rh[lt, pl.ds(s * P2 + 256, 8), :]
                        rh[lt, pl.ds(s * P2 + 264, 8), :] = rh[lt, pl.ds((s + 1) * P2 + 8, 8), :]
                    rh[lt, pl.ds(15 * P2 + 168, 104), :] = jnp.zeros((104, 128), u32)
            return (jnp.minimum(xn + 64, 64 * (NB1 - 1)), hc + 32)
        lax.fori_loop(0, NB1, conv1_step, (zero + 64, zero))

        @pl.when(b == 0)
        def _():
            for part in range(4):
                for c in x_copies(1, part):
                    c.start()
            for piece in range(WPIECE):
                w_copy(w2_hbm, 1, piece).wait()
                _transform_weights(wraw.at[1], wt2, piece)

        run_units(_input_units(load_h(zero), t0))

        def conv2_step(n, c):
            hn, fc = c

            @pl.when(n % 2 == 0)
            def _():
                _conv_block(t0, wt2, acc, store_f(fc), _input_units(load_h(hn), t1))

            @pl.when(n % 2 == 1)
            def _():
                _conv_block(t1, wt2, acc, store_f(fc), _input_units(load_h(hn), t0))
            joint_block(fc, n % 2, b, n)
            return (jnp.minimum(hn + 64, 64 * (NB2 - 1)), fc + 32)
        lax.fori_loop(0, NB2, conv2_step, (zero + 64, zero))
        return carry

    lax.fori_loop(0, B, batch, 0)
    out_wait(0)
    out_wait(1)


def _scratch():
    return [
        pltpu.VMEM((2, 2, 2 * 8 * P1, 128), bf16),
        pltpu.VMEM((2, NSEG * P2, 128), u32),
        pltpu.VMEM((2, NSEG * P3, 128), u32),
        pltpu.VMEM((81, MB // 2, 512), u32),
        pltpu.VMEM((81, MB // 2, 512), u32),
        pltpu.VMEM((2, K, D, D), bf16),
        pltpu.VMEM((81, 256, 256), u32),
        pltpu.VMEM((81, 256, 256), u32),
        pltpu.VMEM((32, MB, D), f32),
        pltpu.VMEM((128, D), u32),
        pltpu.VMEM((128, D), u32),
        pltpu.VMEM((16, D), f32),
        pltpu.VMEM((2, NSEG, 64, U, D), bf16),
        pltpu.SMEM((2,), i32),
        pltpu.SemaphoreType.DMA((2 * WPIECE,)),
        pltpu.SemaphoreType.DMA((4,)),
        pltpu.SemaphoreType.DMA((2,)),
    ]


@jax.jit
def pallas_standalone__seq2seq_rnn_t_joint__speech_kernel(x, w1, w2, g, w_f, w_g, w_o):
    any_spec = pl.BlockSpec(memory_space=pl.ANY)
    vm = pl.BlockSpec(memory_space=pltpu.VMEM)
    return pl.pallas_call(
        _kernel,
        out_shape=jax.ShapeDtypeStruct((B, T2, U, D), bf16),
        in_specs=[pl.BlockSpec(memory_space=pltpu.SMEM), any_spec, any_spec, any_spec, vm, vm, vm, vm],
        out_specs=any_spec,
        scratch_shapes=_scratch(),
        compiler_params=pltpu.CompilerParams(vmem_limit_bytes=120 * 2 ** 20),
    )(np.zeros((1,), np.int32), x, w1, w2, g, w_f, w_g, w_o)
```

```python
import itertools

import numpy as np
import jax
import jax.numpy as jnp
from jax import lax
from jax.experimental import pallas as pl
from jax.experimental.pallas import tpu as pltpu

f32, bf16, u32, i32 = jnp.float32, jnp.bfloat16, jnp.uint32, jnp.int32

B, T, D, K, U = 2, 16000, 256, 31, 8
T1, T2 = T // 2, T // 4
NSEG = 16
G = 4
MB = G * NSEG
P1 = 532
P2 = 274
P3 = 132
NB1, NB2 = 8, 4
XPART = ((0, 80), (80, 144), (144, 336), (336, 528))
W2PIECE = 8
WPIECE = 4
NDOT = 162
LEAD = 6
_C0 = np.float32(np.sqrt(2.0 / np.pi))
_C1 = np.float32(0.044715)
_TG = ((0,), (0, 1), (1,))


def _unpack(w, i):
    return pltpu.unpack_elementwise(w, index=i, packed_dtype=bf16, unpacked_dtype=f32)


def _pack(lo, hi):
    return pltpu.pack_elementwise([lo, hi], packed_dtype=bf16)


def _gelu(x):
    return 0.5 * x * (1.0 + jnp.tanh(_C0 * (x + _C1 * x * x * x)))


def _kar(x0, x1, x2):
    return (x0 - x1, x1, x2 - x1)


def _micro(v):
    w = [_kar(v[i], v[i + 2], v[i + 4]) for i in range(3)]
    out = []
    for ka in range(3):
        out.extend(_kar(w[0][ka], w[1][ka], w[2][ka]))
    return out


def _wtree(get, n):
    if n == 1:
        yield get(0)
        return
    h = n // 2
    lo = [get(j) for j in range(h)]
    yield from _wtree(lambda j: lo[j], h)
    hi = [get(h + j) for j in range(h)]
    mid = [(lo[j][0] + hi[j][0], lo[j][1] + hi[j][1]) for j in range(h)]
    yield from _wtree(lambda j: mid[j], h)
    yield from _wtree(lambda j: hi[j], h)


def _weight_units(w_raw, wt, piece, per):
    wv_ = w_raw.at[:, pl.ds(pl.multiple_of(piece * (16 * per), 16 * per), 16 * per), :]
    units = []
    for ph in range(2):
        wt_ = wt.at[:, pl.ds(pl.multiple_of(ph * 128 + piece * (8 * per), 8 * per), 8 * per), :]
        for r in range(per):
            for nt in range(2):
                def get(j, ph=ph, r=r, nt=nt):
                    tap = 2 * j if ph == 1 else 2 * j - 1
                    if tap < 0:
                        z = jnp.zeros((8, 128), f32)
                        return (z, z)
                    wv = pltpu.bitcast(wv_[tap, pl.ds(16 * r, 16), pl.ds(128 * nt, 128)], u32)
                    return (_unpack(wv, 0), _unpack(wv, 1))
                gen = enumerate(_wtree(get, 16))

                def step(n, gen=gen, wt_=wt_, ph=ph, r=r, nt=nt):
                    def run():
                        for _ in range(n):
                            k, (lo, hi) = next(gen)
                            if k == 0 and ph == 0:
                                continue
                            wt_[k, pl.ds(8 * r, 8), pl.ds(128 * nt, 128)] = _pack(lo, hi)
                    return run
                units.extend(step(9) for _ in range(9))
    return units


def _merge(a, b):
    out, ia, ib = [], 0, 0
    while ia < len(a) or ib < len(b):
        if ib >= len(b) or (ia < len(a) and ia * len(b) <= ib * len(a)):
            out.append(a[ia]); ia += 1
        else:
            out.append(b[ib]); ib += 1
    return out


def _input_units(load, t_out):
    u = {}

    def p1(gq, lt, h, p):
        def run():
            ws = [load(gq, lt, h, p + 4 * j) for j in range(7)]
            for ph in range(2):
                o = _micro([_unpack(w, ph) for w in ws])
                for k in range(9):
                    u[gq, lt, ph, h, k, p] = o[k]
        return run

    def p2(gq, lt, ph, ka):
        def run():
            oa = _micro([u.pop((gq, lt, ph, 0, ka, p)) for p in range(7)])
            ob = _micro([u.pop((gq, lt, ph, 1, ka, p)) for p in range(7)])
            for kb in range(9):
                if ka == 0 and kb == 0 and ph == 0:
                    continue
                t_out[ka * 9 + kb, pl.ds(gq * 8, 8), pl.ds(ph * 256 + lt * 128, 128)] = _pack(oa[kb], ob[kb])
        return run

    cols = [(gq, lt) for gq in range(G) for lt in range(2)]
    seq = []
    for ci in range(len(cols) + 1):
        a = [p1(*cols[ci], h, p) for h in range(2) for p in range(7)] if ci < len(cols) else []
        b = [p2(*cols[ci - 1], ph, ka) for ph in range(2) for ka in range(9)] if ci > 0 else []
        ia = ib = 0
        while ia < len(a) or ib < len(b):
            if ib >= len(b) or (ia < len(a) and ia * len(b) <= ib * len(a)):
                seq.append(a[ia]); ia += 1
            else:
                seq.append(b[ib]); ib += 1
    return seq


def _conv_block(t_in, wt, acc, store, units):
    st = [0, 0]

    def tick():
        st[1] += 1
        want = min(len(units), -(-(st[1] * len(units)) // (NDOT - LEAD)))
        while st[0] < want:
            units[st[0]]()
            st[0] += 1

    groups = list(itertools.product(range(3), repeat=3))
    last = {}
    for gi, (k3, k2, k1) in enumerate(groups):
        for t in itertools.product(_TG[k3], _TG[k2], _TG[k1]):
            last[t] = gi
    seen = set()
    for gi, (k3, k2, k1) in enumerate(groups):
        k = (k3 * 9 + k2 * 3 + k1) * 3
        for nt in range(2):
            cols = slice(nt * 128, (nt + 1) * 128)
            m = []
            for k0 in range(3):
                lo = 256 if k + k0 == 0 else 0
                lhs = pltpu.bitcast(t_in[k + k0, :, lo:], bf16)
                rhs = pltpu.bitcast(wt[k + k0, lo // 2:, cols], bf16)
                m.append(jnp.dot(lhs, rhs, preferred_element_type=f32))
                tick()
            r = (m[0] + m[1], m[1] + m[2])
            for t in itertools.product(_TG[k3], _TG[k2], _TG[k1]):
                a = t[0] * 8 + t[1] * 4 + t[2] * 2
                vals = []
                for a0 in range(2):
                    v = r[a0] if (a + a0, nt) not in seen else acc[a + a0, :, cols] + r[a0]
                    seen.add((a + a0, nt))
                    if last[t] == gi:
                        vals.append(_gelu(v))
                    else:
                        acc[a + a0, :, cols] = v
                if last[t] == gi:
                    for v in range(MB // 8):
                        store(nt, v, a // 2, _pack(vals[0][8 * v:8 * v + 8], vals[1][8 * v:8 * v + 8]))
    while st[0] < len(units):
        units[st[0]]()
        st[0] += 1


def _kernel(zero_ref, x_hbm, w1_hbm, w2_hbm, g_ref, wf_ref, wg_ref, wo_ref, out_hbm,
            rx, rh, rf, t0, t1, wraw, wt1, wt2, acc0, wfp, wop, ge, ob, mode,
            sem_w, sem_x, sem_o):
    zero = zero_ref[0]
    acc = acc0.at[pl.ds(zero, 16)]
    rxw = rx.bitcast(u32)

    def x_copies(b, part):
        cps = []
        lo, hi = XPART[part]
        for s in range(NSEG):
            q0 = max(512 * s - 8 + lo, 0)
            q1 = min(512 * s - 8 + hi, T1)
            if q1 <= q0:
                continue
            loc = q0 - (512 * s - 8)
            for lt in range(2):
                cps.append(pltpu.make_async_copy(
                    x_hbm.at[b, pl.ds(2 * q0, 2 * (q1 - q0)), pl.ds(128 * lt, 128)],
                    rx.at[lt, s % 2, pl.ds(2 * (P1 * (s // 2) + loc), 2 * (q1 - q0)), :],
                    sem_x.at[part]))
        return cps

    def w_copy(w_hbm, i, piece):
        n = D // (WPIECE, W2PIECE)[i]
        rows = pl.ds(pl.multiple_of(piece * n, n), n)
        return pltpu.make_async_copy(w_hbm.at[:, rows, :], wraw.at[i, :, rows, :], sem_w.at[i * WPIECE + piece])

    def out_copy(slot, s, rows, b, t0_):
        return pltpu.make_async_copy(
            ob.at[slot, s, pl.ds(0, rows)], out_hbm.at[b, pl.ds(t0_, rows)], sem_o.at[slot])

    def out_wait(slot):
        m = mode[slot]

        @pl.when(m >= 0)
        def _():
            for s in range(NSEG - 1):
                out_copy(slot, s, 64, 0, 0).wait()

        @pl.when(m == 64)
        def _():
            out_copy(slot, NSEG - 1, 64, 0, 0).wait()

        @pl.when(m == 32)
        def _():
            out_copy(slot, NSEG - 1, 32, 0, 0).wait()

    w_copy(w1_hbm, 0, 0).start()
    for c in x_copies(0, 0):
        c.start()
    for piece in range(1, WPIECE):
        w_copy(w1_hbm, 0, piece).start()

    mode[0] = -1
    mode[1] = -1
    zb = jnp.zeros((16, 128), bf16)
    zw = jnp.zeros((8, 128), u32)
    for lt in range(2):
        rx[lt, 0, pl.ds(0, 16), :] = zb
        rx[lt, 1, pl.ds(2 * P1 * 7 + 656, 400), :] = jnp.zeros((400, 128), bf16)
        rh[lt, pl.ds(0, 8), :] = zw
    wfp[...] = pltpu.bitcast(wf_ref[...], u32)
    wop[...] = pltpu.bitcast(wo_ref[...], u32)
    for b in range(B):
        ge[pl.ds(8 * b, 8), :] = jnp.dot(g_ref[b], wg_ref[...], preferred_element_type=f32)

    def window(ref, idx, base, align, size):
        if isinstance(base, int):
            return ref.at[idx], base
        return ref.at[idx + (pl.ds(pl.multiple_of(base, align), size),)], 0

    def load_x(base):
        def load(gq, lt, h, c):
            view, off = window(rxw, (lt, h), base, 16, 7 * P1 + 80)
            return view[pl.ds(off + 16 * gq + c, 8, stride=P1), :]
        return load

    def load_h(base):
        def load(gq, lt, h, c):
            view, off = window(rh, (lt,), base, 64, 15 * P2 + 80)
            return view[pl.ds(off + h * P2 + 16 * gq + c, 8, stride=2 * P2), :]
        return load

    def store_h(base):
        def store(nt, v, half_a, val):
            view, off = window(rh, (nt,), base, 32, 15 * P2 + 48)
            view[pl.ds(off + 8 * (v % 2) * P2 + 8 + 8 * (v // 2) + half_a, 8, stride=P2), :] = val
        return store

    def store_f(base):
        def store(nt, v, half_a, val):
            view, off = window(rf, (nt,), base, 32, 15 * P3 + 32)
            view[pl.ds(off + 8 * (v % 2) * P3 + 8 * (v // 2) + half_a, 8, stride=P3), :] = val
        return store

    def joint_block(fbase, slot, b, blk):
        out_wait(slot)
        wf = pltpu.bitcast(wfp[...], bf16)
        wo = pltpu.bitcast(wop[...], bf16)
        geb = ge[pl.ds(pl.multiple_of(8 * b, 8), 8), :]

        def fe_of(s):
            lhs = jnp.concatenate(
                [pltpu.bitcast(rf.at[lt, pl.ds(pl.multiple_of(fbase, 32), 15 * P3 + 32), :][pl.ds(s * P3, 32), :], bf16)
                 for lt in range(2)], axis=1)
            return jnp.dot(lhs, wf, preferred_element_type=f32)

        def start_out(s):
            if s < NSEG - 1:
                out_copy(slot, s, 64, b, 256 * s + 64 * blk).start()
                return

            @pl.when(blk < 2)
            def _():
                out_copy(slot, s, 64, b, 256 * s + 64 * blk).start()

            @pl.when(blk == 2)
            def _():
                out_copy(slot, s, 32, b, 256 * s + 128).start()

        fe_next = fe_of(0)
        for s in range(NSEG):
            fe = fe_next
            if s + 1 < NSEG:
                fe_next = fe_of(s + 1)
            for c0 in range(0, 64, 16):
                if c0 == 16 and s > 0:
                    start_out(s - 1)
                rows = [jnp.tanh(jnp.broadcast_to(fe[t:t + 1, :], (8, D)) + geb) for t in range(c0, c0 + 16)]
                j = jnp.concatenate(rows, axis=0).astype(bf16)
                o = jnp.dot(j, wo, preferred_element_type=f32)
                ob[slot, s, pl.ds(c0, 16)] = o.astype(bf16).reshape(16, U, D)
        start_out(NSEG - 1)
        mode[slot] = jnp.where(blk < 2, 64, jnp.where(blk == 2, 32, 0))

    def run_units(units):
        for u in units:
            u()

    def w1_piece(piece, carry):
        w_copy(w1_hbm, 0, piece).wait()

        @pl.when(piece == WPIECE - 2)
        def _():
            for c in x_copies(0, 1):
                c.start()
            w_copy(w2_hbm, 1, 0).start()

        @pl.when(piece == WPIECE - 1)
        def _():
            for part in range(2, 4):
                for c in x_copies(0, part):
                    c.start()
                for p2 in ((1, 2, 3), (4, 5, 6, 7))[part - 2]:
                    w_copy(w2_hbm, 1, p2).start()
        run_units(_weight_units(wraw.at[0], wt1, piece, D // 16 // WPIECE))

        @pl.when(piece == 1)
        def _():
            for c in x_copies(0, 0):
                c.wait()
            run_units(_input_units(load_x(zero), t0))
        return carry
    lax.fori_loop(0, WPIECE, w1_piece, 0)

    def batch(b, carry):
        def conv1_step(n, c):
            xn, hc, wn = c

            @pl.when(b == 0)
            def _():
                w_copy(w2_hbm, 1, n).wait()
            for part, step in ((1, 0), (2, 1), (3, 4)):
                @pl.when(n == step)
                def _(part=part):
                    for cp in x_copies(b, part):
                        cp.wait()

            @pl.when(n % 2 == 0)
            def _():
                _conv_block(t0, wt1, acc, store_h(hc), _merge(
                    _input_units(load_x(xn), t1), _weight_units(wraw.at[1], wt2, wn, 2)))

            @pl.when(n % 2 == 1)
            def _():
                _conv_block(t1, wt1, acc, store_h(hc), _merge(
                    _input_units(load_x(xn), t0), _weight_units(wraw.at[1], wt2, wn, 2)))

            @pl.when(n == NB1 - 1)
            def _():
                for lt in range(2):
                    for s in range(NSEG - 1):
                        rh[lt, pl.ds((s + 1) * P2, 8), :] = rh[lt, pl.ds(s * P2 + 256, 8), :]
                        rh[lt, pl.ds(s * P2 + 264, 8), :] = rh[lt, pl.ds((s + 1) * P2 + 8, 8), :]
                    rh[lt, pl.ds(15 * P2 + 168, 104), :] = jnp.zeros((104, 128), u32)
            return (jnp.minimum(xn + 64, 64 * (NB1 - 1)), hc + 32, wn + 1)
        lax.fori_loop(0, NB1, conv1_step, (zero + 64, zero, zero))

        @pl.when(b == 0)
        def _():
            for part in range(4):
                for cp in x_copies(1, part):
                    cp.start()
        run_units(_input_units(load_h(zero), t0))

        def conv2_step(n, c):
            hn, fc = c

            @pl.when(n % 2 == 0)
            def _():
                _conv_block(t0, wt2, acc, store_f(fc), _input_units(load_h(hn), t1))

            @pl.when(n % 2 == 1)
            def _():
                _conv_block(t1, wt2, acc, store_f(fc), _input_units(load_h(hn), t0))
            joint_block(fc, n % 2, b, n)
            return (jnp.minimum(hn + 64, 64 * (NB2 - 1)), fc + 32)
        lax.fori_loop(0, NB2, conv2_step, (zero + 64, zero))


        @pl.when(b == 0)
        def _():
            for cp in x_copies(1, 0):
                cp.wait()
            run_units(_input_units(load_x(zero), t0))
        return carry

    lax.fori_loop(0, B, batch, 0)
    out_wait(0)
    out_wait(1)


def _scratch():
    return [
        pltpu.VMEM((2, 2, 2 * 8 * P1, 128), bf16),
        pltpu.VMEM((2, NSEG * P2, 128), u32),
        pltpu.VMEM((2, NSEG * P3, 128), u32),
        pltpu.VMEM((81, MB // 2, 512), u32),
        pltpu.VMEM((81, MB // 2, 512), u32),
        pltpu.VMEM((2, K, D, D), bf16),
        pltpu.VMEM((81, 256, 256), u32),
        pltpu.VMEM((81, 256, 256), u32),
        pltpu.VMEM((32, MB, D), f32),
        pltpu.VMEM((128, D), u32),
        pltpu.VMEM((128, D), u32),
        pltpu.VMEM((16, D), f32),
        pltpu.VMEM((2, NSEG, 64, U, D), bf16),
        pltpu.SMEM((2,), i32),
        pltpu.SemaphoreType.DMA((WPIECE + W2PIECE,)),
        pltpu.SemaphoreType.DMA((4,)),
        pltpu.SemaphoreType.DMA((2,)),
    ]


@jax.jit
def pallas_standalone__seq2seq_rnn_t_joint__speech_kernel(x, w1, w2, g, w_f, w_g, w_o):
    any_spec = pl.BlockSpec(memory_space=pl.ANY)
    vm = pl.BlockSpec(memory_space=pltpu.VMEM)
    return pl.pallas_call(
        _kernel,
        out_shape=jax.ShapeDtypeStruct((B, T2, U, D), bf16),
        in_specs=[pl.BlockSpec(memory_space=pltpu.SMEM), any_spec, any_spec, any_spec, vm, vm, vm, vm],
        out_specs=any_spec,
        scratch_shapes=_scratch(),
        compiler_params=pltpu.CompilerParams(vmem_limit_bytes=120 * 2 ** 20),
    )(np.zeros((1,), np.int32), x, w1, w2, g, w_f, w_g, w_o)
```

```python
import itertools

import numpy as np
import jax
import jax.numpy as jnp
from jax import lax
from jax.experimental import pallas as pl
from jax.experimental.pallas import tpu as pltpu

f32, bf16, u32, i32 = jnp.float32, jnp.bfloat16, jnp.uint32, jnp.int32

B, T, D, K, U = 2, 16000, 256, 31, 8
T1, T2 = T // 2, T // 4
NSEG = 16
G = 4
MB = G * NSEG
P1 = 532
P2 = 274
P3 = 132
NB1, NB2 = 8, 4
XPART = ((0, 80), (80, 144), (144, 336), (336, 528))
W2PIECE = 8
WPIECE = 4
NDOT = 162
LEAD = 6
_C0 = np.float32(np.sqrt(2.0 / np.pi))
_C1 = np.float32(0.044715)
_TG = ((0,), (0, 1), (1,))


def _unpack(w, i):
    return lax.bitcast_convert_type(w << 16 if i == 0 else w & np.uint32(0xFFFF0000), f32)


def _pack(lo, hi):
    half = np.uint32(0x8000)
    lo = (lax.bitcast_convert_type(lo, u32) + half) >> 16
    hi = (lax.bitcast_convert_type(hi, u32) + half) & np.uint32(0xFFFF0000)
    return lo | hi


def _gelu(x):
    return 0.5 * x * (1.0 + jnp.tanh(_C0 * (x + _C1 * x * x * x)))


def _kar(x0, x1, x2):
    return (x0 - x1, x1, x2 - x1)


def _micro(v):
    w = [_kar(v[i], v[i + 2], v[i + 4]) for i in range(3)]
    out = []
    for ka in range(3):
        out.extend(_kar(w[0][ka], w[1][ka], w[2][ka]))
    return out


def _wtree(get, n):
    if n == 1:
        yield get(0)
        return
    h = n // 2
    lo = [get(j) for j in range(h)]
    yield from _wtree(lambda j: lo[j], h)
    hi = [get(h + j) for j in range(h)]
    mid = [(lo[j][0] + hi[j][0], lo[j][1] + hi[j][1], None) for j in range(h)]
    yield from _wtree(lambda j: mid[j], h)
    yield from _wtree(lambda j: hi[j], h)


def _weight_units(w_raw, wt, piece, per):
    wv_ = w_raw.at[:, pl.ds(pl.multiple_of(piece * (16 * per), 16 * per), 16 * per), :]
    units = []
    for ph in range(2):
        wt_ = wt.at[:, pl.ds(pl.multiple_of(ph * 128 + piece * (8 * per), 8 * per), 8 * per), :]
        for r in range(per):
            for nt in range(2):
                def get(j, ph=ph, r=r, nt=nt):
                    tap = 2 * j if ph == 1 else 2 * j - 1
                    if tap < 0:
                        z = jnp.zeros((8, 128), f32)
                        return (z, z, None)
                    wv = pltpu.bitcast(wv_[tap, pl.ds(16 * r, 16), pl.ds(128 * nt, 128)], u32)
                    return (_unpack(wv, 0), _unpack(wv, 1), wv)
                gen = enumerate(_wtree(get, 16))

                def step(n, gen=gen, wt_=wt_, ph=ph, r=r, nt=nt):
                    def run():
                        for _ in range(n):
                            k, (lo, hi, raw) = next(gen)
                            if k == 0 and ph == 0:
                                continue
                            wt_[k, pl.ds(8 * r, 8), pl.ds(128 * nt, 128)] = _pack(lo, hi) if raw is None else raw
                    return run
                units.extend(step(9) for _ in range(9))
    return units


def _merge(a, b):
    out, ia, ib = [], 0, 0
    while ia < len(a) or ib < len(b):
        if ib >= len(b) or (ia < len(a) and ia * len(b) <= ib * len(a)):
            out.append(a[ia]); ia += 1
        else:
            out.append(b[ib]); ib += 1
    return out


def _input_units(load, t_out):
    u = {}

    def p1(gq, lt, h, p):
        def run():
            ws = [load(gq, lt, h, p + 4 * j) for j in range(7)]
            for ph in range(2):
                o = _micro([_unpack(w, ph) for w in ws])
                for k in range(9):
                    u[gq, lt, ph, h, k, p] = o[k]
        return run

    def p2(gq, lt, ph, ka):
        def run():
            oa = _micro([u.pop((gq, lt, ph, 0, ka, p)) for p in range(7)])
            ob = _micro([u.pop((gq, lt, ph, 1, ka, p)) for p in range(7)])
            for kb in range(9):
                if ka == 0 and kb == 0 and ph == 0:
                    continue
                for h, o in enumerate((oa, ob)):
                    t_out[ka * 9 + kb, pl.ds(gq * 16 + 8 * h, 8), pl.ds(ph * 256 + lt * 128, 128)] = o[kb]
        return run

    cols = [(gq, lt) for gq in range(G) for lt in range(2)]
    seq = []
    for ci in range(len(cols) + 1):
        a = [p1(*cols[ci], h, p) for h in range(2) for p in range(7)] if ci < len(cols) else []
        b = [p2(*cols[ci - 1], ph, ka) for ph in range(2) for ka in range(9)] if ci > 0 else []
        ia = ib = 0
        while ia < len(a) or ib < len(b):
            if ib >= len(b) or (ia < len(a) and ia * len(b) <= ib * len(a)):
                seq.append(a[ia]); ia += 1
            else:
                seq.append(b[ib]); ib += 1
    return seq


def _conv_block(t_in, wt, acc, store, units):
    st = [0, 0]

    def tick():
        st[1] += 1
        want = min(len(units), -(-(st[1] * len(units)) // (NDOT - LEAD)))
        while st[0] < want:
            units[st[0]]()
            st[0] += 1

    groups = list(itertools.product(range(3), repeat=3))
    last = {}
    for gi, (k3, k2, k1) in enumerate(groups):
        for t in itertools.product(_TG[k3], _TG[k2], _TG[k1]):
            last[t] = gi
    seen = set()
    for gi, (k3, k2, k1) in enumerate(groups):
        k = (k3 * 9 + k2 * 3 + k1) * 3
        for nt in range(2):
            cols = slice(nt * 128, (nt + 1) * 128)
            m = []
            for k0 in range(3):
                lo = 256 if k + k0 == 0 else 0
                lhs = t_in[k + k0, :, lo:].astype(bf16)
                rhs = pltpu.bitcast(wt[k + k0, lo // 2:, cols], bf16)
                m.append(jnp.dot(lhs, rhs, preferred_element_type=f32))
                tick()
            r = (m[0] + m[1], m[1] + m[2])
            for t in itertools.product(_TG[k3], _TG[k2], _TG[k1]):
                a = t[0] * 8 + t[1] * 4 + t[2] * 2
                vals = []
                for a0 in range(2):
                    v = r[a0] if (a + a0, nt) not in seen else acc[a + a0, :, cols] + r[a0]
                    seen.add((a + a0, nt))
                    if last[t] == gi:
                        vals.append(_gelu(v))
                    else:
                        acc[a + a0, :, cols] = v
                if last[t] == gi:
                    for v in range(MB // 8):
                        store(nt, v, a // 2, _pack(vals[0][8 * v:8 * v + 8], vals[1][8 * v:8 * v + 8]))
    while st[0] < len(units):
        units[st[0]]()
        st[0] += 1


def _kernel(zero_ref, x_hbm, w1_hbm, w2_hbm, g_ref, wf_ref, wg_ref, wo_ref, out_hbm,
            rx, rh, rf, t0, t1, wraw, wt1, wt2, acc0, wfp, wop, ge, ob, mode,
            sem_w, sem_x, sem_o):
    zero = zero_ref[0]
    acc = acc0.at[pl.ds(zero, 16)]
    rxw = rx.bitcast(u32)

    def x_copies(b, part):
        cps = []
        lo, hi = XPART[part]
        for s in range(NSEG):
            q0 = max(512 * s - 8 + lo, 0)
            q1 = min(512 * s - 8 + hi, T1)
            if q1 <= q0:
                continue
            loc = q0 - (512 * s - 8)
            for lt in range(2):
                cps.append(pltpu.make_async_copy(
                    x_hbm.at[b, pl.ds(2 * q0, 2 * (q1 - q0)), pl.ds(128 * lt, 128)],
                    rx.at[lt, pl.ds(2 * (P1 * s + loc), 2 * (q1 - q0)), :],
                    sem_x.at[part]))
        return cps

    def w_copy(w_hbm, i, piece):
        n = D // (WPIECE, W2PIECE)[i]
        rows = pl.ds(pl.multiple_of(piece * n, n), n)
        return pltpu.make_async_copy(w_hbm.at[:, rows, :], wraw.at[i, :, rows, :], sem_w.at[i * WPIECE + piece])

    def out_copy(slot, s, rows, b, t0_):
        return pltpu.make_async_copy(
            ob.at[slot, s, pl.ds(0, rows)], out_hbm.at[b, pl.ds(t0_, rows)], sem_o.at[slot])

    def out_wait(slot):
        m = mode[slot]

        @pl.when(m >= 0)
        def _():
            for s in range(NSEG - 1):
                out_copy(slot, s, 64, 0, 0).wait()

        @pl.when(m == 64)
        def _():
            out_copy(slot, NSEG - 1, 64, 0, 0).wait()

        @pl.when(m == 32)
        def _():
            out_copy(slot, NSEG - 1, 32, 0, 0).wait()

    w_copy(w1_hbm, 0, 0).start()
    for c in x_copies(0, 0):
        c.start()
    for piece in range(1, WPIECE):
        w_copy(w1_hbm, 0, piece).start()

    mode[0] = -1
    mode[1] = -1
    zb = jnp.zeros((16, 128), bf16)
    zw = jnp.zeros((8, 128), u32)
    for lt in range(2):
        rx[lt, pl.ds(0, 16), :] = zb
        rx[lt, pl.ds(2 * P1 * 15 + 656, 400), :] = jnp.zeros((400, 128), bf16)
        rh[lt, pl.ds(0, 8), :] = zw
    wfp[...] = pltpu.bitcast(wf_ref[...], u32)
    wop[...] = pltpu.bitcast(wo_ref[...], u32)
    for b in range(B):
        ge[pl.ds(8 * b, 8), :] = jnp.dot(g_ref[b], wg_ref[...], preferred_element_type=f32)

    def window(ref, idx, base, align, size):
        if isinstance(base, int):
            return ref.at[idx], base
        return ref.at[idx + (pl.ds(pl.multiple_of(base, align), size),)], 0

    def load_x(base):
        def load(gq, lt, h, c):
            view, off = window(rxw, (lt,), base, 16, 15 * P1 + 80)
            return view[pl.ds(off + 8 * h * P1 + 16 * gq + c, 8, stride=P1), :]
        return load

    def load_h(base):
        def load(gq, lt, h, c):
            view, off = window(rh, (lt,), base, 64, 15 * P2 + 80)
            return view[pl.ds(off + 8 * h * P2 + 16 * gq + c, 8, stride=P2), :]
        return load

    def store_h(base):
        def store(nt, v, half_a, val):
            view, off = window(rh, (nt,), base, 32, 15 * P2 + 48)
            view[pl.ds(off + 8 * (v % 2) * P2 + 8 + 8 * (v // 2) + half_a, 8, stride=P2), :] = val
        return store

    def store_f(base):
        def store(nt, v, half_a, val):
            view, off = window(rf, (nt,), base, 32, 15 * P3 + 32)
            view[pl.ds(off + 8 * (v % 2) * P3 + 8 * (v // 2) + half_a, 8, stride=P3), :] = val
        return store

    def joint_block(fbase, slot, b, blk):
        out_wait(slot)
        wf = pltpu.bitcast(wfp[...], bf16)
        wo = pltpu.bitcast(wop[...], bf16)
        geb = ge[pl.ds(pl.multiple_of(8 * b, 8), 8), :]

        def fe_of(s):
            lhs = jnp.concatenate(
                [pltpu.bitcast(rf.at[lt, pl.ds(pl.multiple_of(fbase, 32), 15 * P3 + 32), :][pl.ds(s * P3, 32), :], bf16)
                 for lt in range(2)], axis=1)
            return jnp.dot(lhs, wf, preferred_element_type=f32)

        def start_out(s):
            if s < NSEG - 1:
                out_copy(slot, s, 64, b, 256 * s + 64 * blk).start()
                return

            @pl.when(blk < 2)
            def _():
                out_copy(slot, s, 64, b, 256 * s + 64 * blk).start()

            @pl.when(blk == 2)
            def _():
                out_copy(slot, s, 32, b, 256 * s + 128).start()

        fe_next = fe_of(0)
        for s in range(NSEG):
            fe = fe_next
            if s + 1 < NSEG:
                fe_next = fe_of(s + 1)
            for c0 in range(0, 64, 16):
                if c0 == 16 and s > 0:
                    start_out(s - 1)
                rows = [jnp.tanh(jnp.broadcast_to(fe[t:t + 1, :], (8, D)) + geb) for t in range(c0, c0 + 16)]
                j = jnp.concatenate(rows, axis=0).astype(bf16)
                o = jnp.dot(j, wo, preferred_element_type=f32)
                ob[slot, s, pl.ds(c0, 16)] = o.astype(bf16).reshape(16, U, D)
        start_out(NSEG - 1)
        mode[slot] = jnp.where(blk < 2, 64, jnp.where(blk == 2, 32, 0))

    def run_units(units):
        for u in units:
            u()

    def w1_piece(piece, carry):
        w_copy(w1_hbm, 0, piece).wait()

        @pl.when(piece == WPIECE - 2)
        def _():
            for c in x_copies(0, 1):
                c.start()
            w_copy(w2_hbm, 1, 0).start()

        @pl.when(piece == WPIECE - 1)
        def _():
            for part in range(2, 4):
                for c in x_copies(0, part):
                    c.start()
                for p2 in ((1, 2, 3), (4, 5, 6, 7))[part - 2]:
                    w_copy(w2_hbm, 1, p2).start()
        run_units(_weight_units(wraw.at[0], wt1, piece, D // 16 // WPIECE))

        @pl.when(piece == 1)
        def _():
            for c in x_copies(0, 0):
                c.wait()
            run_units(_input_units(load_x(zero), t0))
        return carry
    lax.fori_loop(0, WPIECE, w1_piece, 0)

    def batch(b, carry):
        def conv1_step(n, c):
            xn, hc, wn = c

            @pl.when(b == 0)
            def _():
                w_copy(w2_hbm, 1, n).wait()
            for part, step in ((1, 0), (2, 1), (3, 4)):
                @pl.when(n == step)
                def _(part=part):
                    for cp in x_copies(b, part):
                        cp.wait()

            @pl.when(n % 2 == 0)
            def _():
                _conv_block(t0, wt1, acc, store_h(hc), _merge(
                    _input_units(load_x(xn), t1), _weight_units(wraw.at[1], wt2, wn, 2)))

            @pl.when(n % 2 == 1)
            def _():
                _conv_block(t1, wt1, acc, store_h(hc), _merge(
                    _input_units(load_x(xn), t0), _weight_units(wraw.at[1], wt2, wn, 2)))

            @pl.when(n == NB1 - 1)
            def _():
                for lt in range(2):
                    for s in range(NSEG - 1):
                        rh[lt, pl.ds((s + 1) * P2, 8), :] = rh[lt, pl.ds(s * P2 + 256, 8), :]
                        rh[lt, pl.ds(s * P2 + 264, 8), :] = rh[lt, pl.ds((s + 1) * P2 + 8, 8), :]
                    rh[lt, pl.ds(15 * P2 + 168, 104), :] = jnp.zeros((104, 128), u32)
            return (jnp.minimum(xn + 64, 64 * (NB1 - 1)), hc + 32, wn + 1)
        lax.fori_loop(0, NB1, conv1_step, (zero + 64, zero, zero))

        @pl.when(b == 0)
        def _():
            for part in range(4):
                for cp in x_copies(1, part):
                    cp.start()

        run_units(_input_units(load_h(zero), t0))

        def conv2_step(n, c):
            hn, fc = c

            @pl.when(n % 2 == 0)
            def _():
                _conv_block(t0, wt2, acc, store_f(fc), _input_units(load_h(hn), t1))

            @pl.when(n % 2 == 1)
            def _():
                _conv_block(t1, wt2, acc, store_f(fc), _input_units(load_h(hn), t0))
            joint_block(fc, n % 2, b, n)
            return (jnp.minimum(hn + 64, 64 * (NB2 - 1)), fc + 32)
        lax.fori_loop(0, NB2, conv2_step, (zero + 64, zero))

        @pl.when(b == 0)
        def _():
            for cp in x_copies(1, 0):
                cp.wait()
            run_units(_input_units(load_x(zero), t0))
        return carry

    lax.fori_loop(0, B, batch, 0)
    out_wait(0)
    out_wait(1)


def _scratch():
    return [
        pltpu.VMEM((2, 2 * NSEG * P1, 128), bf16),
        pltpu.VMEM((2, NSEG * P2, 128), u32),
        pltpu.VMEM((2, NSEG * P3, 128), u32),
        pltpu.VMEM((81, MB, 512), f32),
        pltpu.VMEM((81, MB, 512), f32),
        pltpu.VMEM((2, K, D, D), bf16),
        pltpu.VMEM((81, 256, 256), u32),
        pltpu.VMEM((81, 256, 256), u32),
        pltpu.VMEM((32, MB, D), f32),
        pltpu.VMEM((128, D), u32),
        pltpu.VMEM((128, D), u32),
        pltpu.VMEM((16, D), f32),
        pltpu.VMEM((2, NSEG, 64, U, D), bf16),
        pltpu.SMEM((2,), i32),
        pltpu.SemaphoreType.DMA((WPIECE + W2PIECE,)),
        pltpu.SemaphoreType.DMA((4,)),
        pltpu.SemaphoreType.DMA((2,)),
    ]


@jax.jit
def pallas_standalone__seq2seq_rnn_t_joint__speech_kernel(x, w1, w2, g, w_f, w_g, w_o):
    any_spec = pl.BlockSpec(memory_space=pl.ANY)
    vm = pl.BlockSpec(memory_space=pltpu.VMEM)
    return pl.pallas_call(
        _kernel,
        out_shape=jax.ShapeDtypeStruct((B, T2, U, D), bf16),
        in_specs=[pl.BlockSpec(memory_space=pltpu.SMEM), any_spec, any_spec, any_spec, vm, vm, vm, vm],
        out_specs=any_spec,
        scratch_shapes=_scratch(),
        compiler_params=pltpu.CompilerParams(vmem_limit_bytes=120 * 2 ** 20),
    )(np.zeros((1,), np.int32), x, w1, w2, g, w_f, w_g, w_o)
```
